```python
import os as _os
_os.environ.setdefault("JAX_PLATFORMS", "cpu")
import jax
import jax.numpy as jnp

def _softmax(x, axis=-1):
    return jax.nn.softmax(x, axis=axis)
def _gelu(x):
    return jax.nn.gelu(x, approximate=True)
def _silu(x):
    return jax.nn.silu(x)
def _sigmoid(x):
    return jax.nn.sigmoid(x)
def _layernorm(x, axis=-1, eps=1e-5):
    m = jnp.mean(x, axis=axis, keepdims=True)
    v = jnp.var(x, axis=axis, keepdims=True)
    return (x - m) / jnp.sqrt(v + eps)
def _scatter_add(tgt, idx, src, axis=0):
    return tgt.at[idx].add(src)
def _segment_sum(src, seg, n):
    return jax.ops.segment_sum(src, seg, n)
class _Rng:
    def __init__(self, key):
        self._k = key
    def _next(self):
        self._k, sub = jax.random.split(self._k)
        return sub
    def normal(self, shape):
        return jax.random.normal(self._next(), shape, dtype=jnp.bfloat16)
    def randint(self, lo, hi, shape):
        return jax.random.randint(self._next(), shape, lo, hi, dtype=jnp.int32)
    def uniform(self, shape, lo=0.0, hi=1.0):
        return jax.random.uniform(self._next(), shape, jnp.bfloat16, lo, hi)
    def permutation(self, n):
        return jax.random.permutation(self._next(), n)


kernel_name = 'standalone__dense_activation_gelu__prompt'

def setup_inputs():
    _rng = _Rng(jax.random.key(int.from_bytes(__import__("os").urandom(4), "little")))
    _w = (lambda a: (lambda t: t.astype(jnp.bfloat16) if jnp.issubdtype(t.dtype, jnp.floating) else t)(jnp.asarray(a)))
    B, S, D, F = 1, 2048, 640, 1728
    return {
        "x": _w((lambda *s: _rng.normal(s) * 0.05)(B, S, D)),
        "w1": _w((lambda *s: _rng.normal(s) * 0.05)(D, F) * (D ** -0.5)),
        "b1": _w((lambda *s: _rng.normal(s) * 0.05)(F) * 0.01),
        "w2": _w((lambda *s: _rng.normal(s) * 0.05)(F, D) * (F ** -0.5)),
        "b2": _w((lambda *s: _rng.normal(s) * 0.05)(D) * 0.01),
    }

def reference(x, w1, b1, w2, b2):
    h = jnp.einsum("bsd,df->bsf", x, w1) + b1
    h = _gelu(h)
    return jnp.einsum("bsf,fd->bsd", h, w2) + b2
```

```python
import jax
import jax.numpy as jnp
import jax.experimental.pallas as pl
import jax.experimental.pallas.tpu as pltpu

_NT = (((1,), (1,)), ((), ()))


def _msplit(fn, a, n):
    if n == 1:
        return fn(a)
    r = a.shape[0] // n
    return jnp.concatenate([fn(a[i * r:(i + 1) * r]) for i in range(n)], axis=0)


@jax.jit
def pallas_standalone__dense_activation_gelu__prompt_kernel(x, w1, b1, w2, b2):
    B, S, D = x.shape
    F = w1.shape[1]
    FM = (F // 128) * 128
    tm0, fa, tm, last = 768, 1024, 384, 128
    ksteps = ((0, 1), (1, 3), (3, 5))
    nk = len(ksteps)
    blocks = [(r, tm) for r in range(tm0, S - last, tm)] + [(S - last, last)]
    SXK = 0; SWK = SXK + nk; SB1 = SWK + nk; SW1R = SB1 + 1; SW2 = SW1R + 1
    SB2 = SW2 + 1; SXR = SB2 + 1; SO = SXR + 1
    nsem = SO + 1 + len(blocks)

    def body(x_hbm, w1t_hbm, b1_hbm, w2_hbm, b2_hbm, o_hbm, x_v, w1_v, w2_v, b1_v, b2_v, o_v, h_v, sem):
        def cp(src, dst, s, e, k, c0=None, c1=None):
            if c0 is None:
                return pltpu.make_async_copy(src.at[s:e], dst.at[s:e], sem.at[k])
            return pltpu.make_async_copy(src.at[s:e, c0:c1], dst.at[s:e, c0:c1], sem.at[k])
        cxk = [cp(x_hbm, x_v, 0, tm0, SXK + i, a * 128, b * 128) for i, (a, b) in enumerate(ksteps)]
        cwk = [cp(w1t_hbm, w1_v, 0, fa, SWK + i, a * 128, b * 128) for i, (a, b) in enumerate(ksteps)]
        cb1 = pltpu.make_async_copy(b1_hbm, b1_v, sem.at[SB1])
        cw1r = cp(w1t_hbm, w1_v, fa, F, SW1R)
        cw2 = cp(w2_hbm, w2_v, 0, F, SW2)
        cb2 = pltpu.make_async_copy(b2_hbm, b2_v, sem.at[SB2])
        cxr = cp(x_hbm, x_v, tm0, S, SXR)
        outs = [cp(o_v, o_hbm, 0, tm0, SO)] + [cp(o_v, o_hbm, r, r + n, SO + 1 + i) for i, (r, n) in enumerate(blocks)]

        for i in range(nk):
            cxk[i].start(); cwk[i].start()
            if i == 0:
                cb1.start()
        cw1r.start(); cw2.start(); cb2.start(); cxr.start()

        def ldb1(): return b1_v[...].astype(jnp.float32).reshape(1, F)
        def ldb2(): return b2_v[...].astype(jnp.float32).reshape(1, D)
        def act(h, b): return jax.nn.gelu(h + b, approximate=True).astype(jnp.bfloat16)
        def nt(a, b): return jax.lax.dot_general(a, b, _NT, preferred_element_type=jnp.float32)
        def mm1_tail(xb, bias):
            return act(nt(w1_v[FM:F, :], xb).T, bias[:, FM:F])
        def mm2(g, s, e, n=1):
            return _msplit(lambda gg: jnp.dot(gg, w2_v[s:e, :], preferred_element_type=jnp.float32), g[:, s:e], n)

        for i, (a, b) in enumerate(ksteps):
            lastk = (i == nk - 1)
            cxk[i].wait(); cwk[i].wait()
            if i == 0:
                cb1.wait()
            if lastk:
                cw1r.wait()
            c0, c1 = a * 128, b * 128
            p = nt(x_v[0:tm0, c0:c1], w1_v[0:fa, c0:c1])
            if i == 0:
                h_v[...] = p
            elif not lastk:
                h_v[...] += p
            else:
                bias = ldb1()
                xb = x_v[0:tm0, :]
                g = jnp.concatenate([
                    act(h_v[...] + p, bias[:, 0:fa]),
                    act(nt(xb, w1_v[fa:FM, :]), bias[:, fa:FM]),
                    mm1_tail(xb, bias)], axis=1)
        cw2.wait(); cb2.wait(); cxr.wait()
        acc = mm2(g, 0, 1536) + mm2(g, 1536, F, 2)
        o_v[0:tm0, :] = (acc + ldb2()).astype(o_v.dtype)
        outs[0].start()
        for i, (r, n) in enumerate(blocks):
            xb = x_v[r:r + n, :]
            bias = ldb1()
            g = jnp.concatenate([act(nt(xb, w1_v[0:FM, :]), bias[:, 0:FM]), mm1_tail(xb, bias)], axis=1)
            o_v[r:r + n, :] = (mm2(g, 0, F) + ldb2()).astype(o_v.dtype)
            outs[1 + i].start()
        for c in outs:
            c.wait()

    hbm = pl.BlockSpec(memory_space=pltpu.HBM)
    out = pl.pallas_call(
        body, in_specs=[hbm] * 5, out_specs=hbm,
        out_shape=jax.ShapeDtypeStruct((B * S, D), x.dtype),
        scratch_shapes=[
            pltpu.VMEM((S, D), jnp.bfloat16), pltpu.VMEM((F, D), jnp.bfloat16), pltpu.VMEM((F, D), jnp.bfloat16),
            pltpu.VMEM((F,), jnp.bfloat16), pltpu.VMEM((D,), jnp.bfloat16), pltpu.VMEM((S, D), jnp.bfloat16),
            pltpu.VMEM((tm0, fa), jnp.float32),
            pltpu.SemaphoreType.DMA((nsem,)),
        ],
        compiler_params=pltpu.CompilerParams(vmem_limit_bytes=100 * 1024 * 1024, disable_semaphore_checks=True),
    )(x.reshape(B * S, D), w1.T, b1, w2, b2)
    return out.reshape(B, S, D)
```

```python
import jax
import jax.numpy as jnp
import jax.experimental.pallas as pl
import jax.experimental.pallas.tpu as pltpu

_NT = (((1,), (1,)), ((), ()))


def _row_split(fn, a, n):
    if n == 1:
        return fn(a)
    r = a.shape[0] // n
    return jnp.concatenate([fn(a[i * r:(i + 1) * r]) for i in range(n)], axis=0)


@jax.jit
def pallas_standalone__dense_activation_gelu__prompt_kernel(x, w1, b1, w2, b2):
    B, S, D = x.shape
    F = w1.shape[1]
    M = B * S
    FM = (F // 128) * 128
    TM0 = 768
    half = ((0, 512, 1), (512, 1024, 1))
    ksteps = (((0, 1), tuple((f, f + 128, 4) for f in range(0, 1024, 128))),
              ((1, 2), half), ((2, 3), half), ((3, 5), half))
    FA = 1024
    full = ((FA, 1536), (1536, FM))
    rows = ((TM0, 896), (TM0 + 896, 384))
    pieces = ((0, TM0, 896), (1, 1664, 160), (1, 1824, 128), (1, 1952, 64), (1, 2016, 32))
    nk = len(ksteps)
    nsem = nk + sum(len(fs) for _, fs in ksteps) + len(full) + 1 + 1 + 2 + len(rows)

    def body(x_hbm, w1t_hbm, b1_hbm, w2_hbm, b2_hbm, o_hbm,
             x_v, w1_v, w2_v, b1_v, b2_v, o_v, h_v, sem, osem):
        cnt = [0]

        def cp(src, dst, s=None, e=None, c0=None, c1=None):
            k = cnt[0]
            cnt[0] += 1
            if s is None:
                return pltpu.make_async_copy(src, dst, sem.at[k])
            if c0 is None:
                return pltpu.make_async_copy(src.at[s:e], dst.at[s:e], sem.at[k])
            return pltpu.make_async_copy(src.at[s:e, c0:c1], dst.at[s:e, c0:c1], sem.at[k])

        cx = [cp(x_hbm, x_v, 0, TM0, a * 128, b * 128) for ((a, b), _) in ksteps]
        cw = [[cp(w1t_hbm, w1_v, f0, f1, a * 128, b * 128) for (f0, f1, _) in fs] for ((a, b), fs) in ksteps]
        cf = [cp(w1t_hbm, w1_v, s, e) for (s, e) in full]
        ct = cp(w1t_hbm, w1_v, FM, F)
        c2 = cp(w2_hbm, w2_v, 0, F)
        cb1 = cp(b1_hbm, b1_v)
        cb2 = cp(b2_hbm, b2_v)
        cxr = [cp(x_hbm, x_v, r, r + n) for (r, n) in rows]
        out0 = pltpu.make_async_copy(o_v.at[0:TM0], o_hbm.at[0:TM0], osem.at[0])
        outs = [pltpu.make_async_copy(o_v.at[s:s + n], o_hbm.at[s:s + n], osem.at[1 + i])
                for i, (_, s, n) in enumerate(pieces)]

        for i in range(nk):
            cw[i][0].start()
            cx[i].start()
            for c in cw[i][1:]:
                c.start()
            if i == 0:
                cb1.start()
        for c in cf:
            c.start()
        ct.start()
        c2.start()
        cb2.start()
        for c in cxr:
            c.start()

        def ldb1():
            return b1_v[...].astype(jnp.float32).reshape(1, F)

        def ldb2():
            return b2_v[...].astype(jnp.float32).reshape(1, D)

        def act(h, b):
            return jax.nn.gelu(h + b, approximate=True).astype(jnp.bfloat16)

        def nt(a, b):
            return jax.lax.dot_general(a, b, _NT, preferred_element_type=jnp.float32)

        def mm1_main(xb, s, e, bias):
            return act(nt(xb, w1_v[s:e, :]), bias[:, s:e])

        def mm1_tail(xb, bias):
            return act(nt(w1_v[FM:F, :], xb).T, bias[:, FM:F])

        def mm2(g):
            return jnp.dot(g, w2_v[...], preferred_element_type=jnp.float32)

        xs, parts = [], []
        for i, ((a, b), fs) in enumerate(ksteps):
            c0, c1 = a * 128, b * 128
            for j, (f0, f1, n) in enumerate(fs):
                cw[i][j].wait()
                if j == 0:
                    cx[i].wait()
                    xs.append(x_v[0:TM0, c0:c1])
                    if i == 1:
                        cb1.wait()
                p = _row_split(lambda xx: nt(xx, w1_v[f0:f1, c0:c1]), xs[i], n)
                if i == 0:
                    h_v[:, f0:f1] = p
                elif i < nk - 1:
                    h_v[:, f0:f1] += p
                else:
                    parts.append(act(h_v[:, f0:f1] + p, ldb1()[:, f0:f1]))
        xb = jnp.concatenate(xs, axis=1)
        bias = ldb1()
        for j, (s, e) in enumerate(full):
            cf[j].wait()
            parts.append(mm1_main(xb, s, e, bias))
        ct.wait()
        parts.append(mm1_tail(xb, bias))
        g = jnp.concatenate(parts, axis=1)
        cxr[0].wait()
        c2.wait()
        cb2.wait()
        o_v[0:TM0, :] = (mm2(g) + ldb2()).astype(o_v.dtype)
        out0.start()
        pi = 0
        for j, (r0, n) in enumerate(rows):
            xb = x_v[r0:r0 + n, :]
            bias = ldb1()
            g = jnp.concatenate([mm1_main(xb, 0, FM, bias), mm1_tail(xb, bias)], axis=1)
            if j + 1 < len(rows):
                cxr[j + 1].wait()
            while pi < len(pieces) and pieces[pi][0] == j:
                _, s, q = pieces[pi]
                o_v[s:s + q, :] = (mm2(g[s - r0:s - r0 + q, :]) + ldb2()).astype(o_v.dtype)
                outs[pi].start()
                pi += 1
        out0.wait()
        for c in outs:
            c.wait()

    hbm = pl.BlockSpec(memory_space=pltpu.HBM)
    out = pl.pallas_call(
        body,
        in_specs=[hbm] * 5,
        out_specs=hbm,
        out_shape=jax.ShapeDtypeStruct((M, D), x.dtype),
        scratch_shapes=[
            pltpu.VMEM((M, D), jnp.bfloat16), pltpu.VMEM((F, D), jnp.bfloat16), pltpu.VMEM((F, D), jnp.bfloat16),
            pltpu.VMEM((F,), jnp.bfloat16), pltpu.VMEM((D,), jnp.bfloat16), pltpu.VMEM((M, D), jnp.bfloat16),
            pltpu.VMEM((TM0, FA), jnp.float32),
            pltpu.SemaphoreType.DMA((nsem,)), pltpu.SemaphoreType.DMA((1 + len(pieces),)),
        ],
        compiler_params=pltpu.CompilerParams(
            vmem_limit_bytes=100 * 1024 * 1024,
            disable_semaphore_checks=True,
            flags={"XLA_TPU_RESCHEDULE_DMA_DONES": True},
        ),
    )(x.reshape(M, D), w1.T, b1, w2, b2)
    return out.reshape(B, S, D)
```

```python
import jax
import jax.numpy as jnp
from jax.experimental import pallas as pl
from jax.experimental.pallas import tpu as pltpu

_NT = (((1,), (1,)), ((), ()))

_T = 128
_TM0 = 896
_X0_PIECES = (448, 448)
_FA = 1024
_MID = ((0, 512, 1), (512, 768, 2), (768, 1024, 2))
_K_STEPS = (((1, 2), _MID), ((2, 3), _MID), ((3, 5), ((0, 512, 1), (512, 1024, 1))))
_FULL = ((1024, 1536), (1536, 1664))
_BLOCKS = (768, 384)
_LAST_PIECES = (192, 96, 64, 32)


def _row_split(fn, a, n):
    if n == 1:
        return fn(a)
    r = a.shape[0] // n
    return jnp.concatenate([fn(a[i * r:(i + 1) * r]) for i in range(n)], axis=0)


def _spans(start, sizes):
    out = []
    for n in sizes:
        out.append((start, start + n))
        start += n
    return out


def _make_kernel(M, D, F):
    FM = (F // _T) * _T
    x0_pieces = _spans(0, _X0_PIECES)
    blocks = _spans(_TM0, _BLOCKS)
    out_pieces = [(j, s, e) for j, (s, e) in enumerate(blocks[:-1])]
    out_pieces += [(len(blocks) - 1, s, e) for (s, e) in _spans(blocks[-1][0], _LAST_PIECES)]
    assert x0_pieces[-1][1] == _TM0 and blocks[-1][1] == M and out_pieces[-1][2] == M
    assert D == 5 * _T and _K_STEPS[-1][0][1] * _T == D and _FULL[-1][1] == FM and 0 < F - FM < _T
    first_tiles = [(f, f + _T) for f in range(0, _FA, _T)]
    n_in = (len(x0_pieces) + len(first_tiles) + sum(1 + len(fs) for _, fs in _K_STEPS)
            + len(_FULL) + 2 + 2 + len(blocks))
    n_out = 1 + len(out_pieces)

    def kernel(x_hbm, w1t_hbm, b1_hbm, w2_hbm, b2_hbm, o_hbm,
               x_v, w1_v, w2_v, b1_v, b2_v, o_v, h_v, in_sem, out_sem):

        def work():
            used = [0]

            def load(src, dst, rows=None, cols=None):
                k = used[0]
                used[0] += 1
                if rows is None:
                    return pltpu.make_async_copy(src, dst, in_sem.at[k])
                r = slice(*rows)
                if cols is None:
                    return pltpu.make_async_copy(src.at[r], dst.at[r], in_sem.at[k])
                c = slice(*cols)
                return pltpu.make_async_copy(src.at[r, c], dst.at[r, c], in_sem.at[k])

            c_x0 = [load(x_hbm, x_v, rows, (0, _T)) for rows in x0_pieces]
            c_w0 = [load(w1t_hbm, w1_v, rows, (0, _T)) for rows in first_tiles]
            c_xk = [load(x_hbm, x_v, (0, _TM0), (a * _T, b * _T)) for (a, b), _ in _K_STEPS]
            c_wk = [[load(w1t_hbm, w1_v, (f0, f1), (a * _T, b * _T)) for (f0, f1, _) in fs]
                    for (a, b), fs in _K_STEPS]
            c_full = [load(w1t_hbm, w1_v, rows) for rows in _FULL]
            c_tail = load(w1t_hbm, w1_v, (FM, F))
            c_w2 = load(w2_hbm, w2_v, (0, F))
            c_b1 = load(b1_hbm, b1_v)
            c_b2 = load(b2_hbm, b2_v)
            c_xb = [load(x_hbm, x_v, rows) for rows in blocks]
            assert used[0] == n_in
            outs = [pltpu.make_async_copy(o_v.at[s:e], o_hbm.at[s:e], out_sem.at[i])
                    for i, (_, s, e) in enumerate([(None, 0, _TM0)] + out_pieces)]

            c_w0[0].start()
            c_x0[0].start()
            c_w0[1].start()
            c_b1.start()
            for c in c_w0[2:] + c_x0[1:]:
                c.start()
            for cx, cws in zip(c_xk, c_wk):
                cws[0].start()
                cx.start()
                for c in cws[1:]:
                    c.start()
            for c in c_full + [c_tail, c_w2, c_b2] + c_xb:
                c.start()

            def bias1():
                return b1_v[...].astype(jnp.float32).reshape(1, F)

            def bias2():
                return b2_v[...].astype(jnp.float32).reshape(1, D)

            def act(h, b):
                return jax.nn.gelu(h + b, approximate=True).astype(jnp.bfloat16)

            def dot_nt(a, b):
                return jax.lax.dot_general(a, b, _NT, preferred_element_type=jnp.float32)

            def hidden(xb, f0, f1):
                return act(dot_nt(xb, w1_v[f0:f1, :]), bias1()[:, f0:f1])

            def hidden_tail(xb):
                return act(dot_nt(w1_v[FM:F, :], xb).T, bias1()[:, FM:F])

            def project(g):
                return (jnp.dot(g, w2_v[...], preferred_element_type=jnp.float32) + bias2()).astype(o_v.dtype)

            x_cols = []
            pieces = []
            for p, (r0, r1) in enumerate(x0_pieces):
                for t, (f0, f1) in enumerate(first_tiles):
                    if p == 0:
                        c_w0[t].wait()
                        if t == 4:
                            c_b1.wait()
                    if t == 0:
                        c_x0[p].wait()
                        pieces.append(x_v[r0:r1, 0:_T])
                    h_v[r0:r1, f0:f1] = _row_split(lambda xx: dot_nt(xx, w1_v[f0:f1, 0:_T]), pieces[-1], 4)
            x_cols.append(jnp.concatenate(pieces, axis=0))

            g_parts = []
            for i, ((a, b), fs) in enumerate(_K_STEPS):
                c0, c1 = a * _T, b * _T
                last = i == len(_K_STEPS) - 1
                for j, (f0, f1, n) in enumerate(fs):
                    c_wk[i][j].wait()
                    if j == 0:
                        c_xk[i].wait()
                        x_cols.append(x_v[0:_TM0, c0:c1])
                    p = _row_split(lambda xx: dot_nt(xx, w1_v[f0:f1, c0:c1]), x_cols[-1], n)
                    if last:
                        g_parts.append(act(h_v[:, f0:f1] + p, bias1()[:, f0:f1]))
                    else:
                        h_v[:, f0:f1] += p

            xb = jnp.concatenate(x_cols, axis=1)
            for c, (f0, f1) in zip(c_full, _FULL):
                c.wait()
                g_parts.append(hidden(xb, f0, f1))
            c_tail.wait()
            g_parts.append(hidden_tail(xb))
            g = jnp.concatenate(g_parts, axis=1)
            c_w2.wait()
            c_b2.wait()
            o_v[0:_TM0, :] = project(g)
            outs[0].start()

            for j, (r0, r1) in enumerate(blocks):
                c_xb[j].wait()
                xb = x_v[r0:r1, :]
                g = jnp.concatenate([hidden(xb, 0, FM), hidden_tail(xb)], axis=1)
                for i, (blk, s, e) in enumerate(out_pieces):
                    if blk == j:
                        o_v[s:e, :] = project(g[s - r0:e - r0, :])
                        outs[1 + i].start()

            for c in outs:
                c.wait()

        def trip(t, carry):
            pl.when(t == 0)(work)
            return carry

        jax.lax.fori_loop(0, 2, trip, 0)

    return kernel, n_in, n_out


@jax.jit
def pallas_standalone__dense_activation_gelu__prompt_kernel(x, w1, b1, w2, b2):
    B, S, D = x.shape
    F = w1.shape[1]
    M = B * S
    kernel, n_in, n_out = _make_kernel(M, D, F)
    hbm = pl.BlockSpec(memory_space=pltpu.HBM)
    out = pl.pallas_call(
        kernel,
        in_specs=[hbm] * 5,
        out_specs=hbm,
        out_shape=jax.ShapeDtypeStruct((M, D), x.dtype),
        scratch_shapes=[
            pltpu.VMEM((M, D), x.dtype),
            pltpu.VMEM((F, D), w1.dtype),
            pltpu.VMEM((F, D), w2.dtype),
            pltpu.VMEM((F,), b1.dtype),
            pltpu.VMEM((D,), b2.dtype),
            pltpu.VMEM((M, D), x.dtype),
            pltpu.VMEM((_TM0, _FA), jnp.float32),
            pltpu.SemaphoreType.DMA((n_in,)),
            pltpu.SemaphoreType.DMA((n_out,)),
        ],
        compiler_params=pltpu.CompilerParams(
            vmem_limit_bytes=100 * 1024 * 1024,
            disable_semaphore_checks=True,
            flags={"XLA_TPU_RESCHEDULE_DMA_DONES": True},
        ),
    )(x.reshape(M, D), w1.T, b1, w2, b2)
    return out.reshape(B, S, D)
```

```python
import jax
import jax.numpy as jnp
from jax.experimental import pallas as pl
from jax.experimental.pallas import tpu as pltpu

_NT = (((1,), (1,)), ((), ()))

_T = 128
_TM0 = 896
_X0_PIECES = (448, 448)
_FA = 1024
_MID = ((0, 512, 1), (512, 768, 2), (768, 1024, 2))
_K_STEPS = (((1, 2), _MID), ((2, 3), _MID), ((3, 5), ((0, 512, 1), (512, 1024, 1))))
_FULL = ((1024, 1536), (1536, 1664))
_BLOCKS = (768, 384)
_LAST_PIECES = (192, 96, 64, 32)
_LAST_COLS = ((0, 512), (512, 640))


def _row_split(fn, a, n):
    if n == 1:
        return fn(a)
    r = a.shape[0] // n
    return jnp.concatenate([fn(a[i * r:(i + 1) * r]) for i in range(n)], axis=0)


def _spans(start, sizes):
    out = []
    for n in sizes:
        out.append((start, start + n))
        start += n
    return out


def _make_kernel(M, D, F):
    FM = (F // _T) * _T
    x0_pieces = _spans(0, _X0_PIECES)
    blocks = _spans(_TM0, _BLOCKS)
    out_pieces = [(j, s, e) for j, (s, e) in enumerate(blocks[:-1])]
    out_pieces += [(len(blocks) - 1, s, e) for (s, e) in _spans(blocks[-1][0], _LAST_PIECES)]
    assert x0_pieces[-1][1] == _TM0 and blocks[-1][1] == M and out_pieces[-1][2] == M
    assert _LAST_COLS[0][0] == 0 and _LAST_COLS[-1][1] == D
    assert D == 5 * _T and _K_STEPS[-1][0][1] * _T == D and _FULL[-1][1] == FM and 0 < F - FM < _T
    first_tiles = [(f, f + _T) for f in range(0, _FA, _T)]
    n_in = (len(x0_pieces) + len(first_tiles) + sum(1 + len(fs) for _, fs in _K_STEPS)
            + len(_FULL) + 2 + 2 + len(blocks))
    n_out = len(out_pieces) + len(_LAST_COLS)

    def kernel(x_hbm, w1t_hbm, b1_hbm, w2_hbm, b2_hbm, o_hbm,
               x_v, w1_v, w2_v, b1_v, b2_v, o_v, h_v, in_sem, out_sem):

        def work():
            used = [0]

            def load(src, dst, rows=None, cols=None):
                k = used[0]
                used[0] += 1
                if rows is None:
                    return pltpu.make_async_copy(src, dst, in_sem.at[k])
                r = slice(*rows)
                if cols is None:
                    return pltpu.make_async_copy(src.at[r], dst.at[r], in_sem.at[k])
                c = slice(*cols)
                return pltpu.make_async_copy(src.at[r, c], dst.at[r, c], in_sem.at[k])

            c_x0 = [load(x_hbm, x_v, rows, (0, _T)) for rows in x0_pieces]
            c_w0 = [load(w1t_hbm, w1_v, rows, (0, _T)) for rows in first_tiles]
            c_xk = [load(x_hbm, x_v, (0, _TM0), (a * _T, b * _T)) for (a, b), _ in _K_STEPS]
            c_wk = [[load(w1t_hbm, w1_v, (f0, f1), (a * _T, b * _T)) for (f0, f1, _) in fs]
                    for (a, b), fs in _K_STEPS]
            c_full = [load(w1t_hbm, w1_v, rows) for rows in _FULL]
            c_tail = load(w1t_hbm, w1_v, (FM, F))
            c_w2 = load(w2_hbm, w2_v, (0, F))
            c_b1 = load(b1_hbm, b1_v)
            c_b2 = load(b2_hbm, b2_v)
            c_xb = [load(x_hbm, x_v, rows) for rows in blocks]
            assert used[0] == n_in
            outs = [pltpu.make_async_copy(o_v.at[s:e], o_hbm.at[s:e], out_sem.at[i])
                    for i, (_, s, e) in enumerate([(None, 0, _TM0)] + out_pieces[:-1])]
            _, s_last, e_last = out_pieces[-1]
            outs_last = [pltpu.make_async_copy(o_v.at[s_last:e_last, n0:n1], o_hbm.at[s_last:e_last, n0:n1],
                                               out_sem.at[len(outs) + q])
                         for q, (n0, n1) in enumerate(_LAST_COLS)]

            c_w0[0].start()
            c_x0[0].start()
            c_w0[1].start()
            c_b1.start()
            for c in c_w0[2:] + c_x0[1:]:
                c.start()
            for cx, cws in zip(c_xk, c_wk):
                cws[0].start()
                cx.start()
                for c in cws[1:]:
                    c.start()
            for c in c_full + [c_tail, c_w2, c_b2] + c_xb:
                c.start()

            def bias1():
                return b1_v[...].astype(jnp.float32).reshape(1, F)

            def bias2():
                return b2_v[...].astype(jnp.float32).reshape(1, D)

            def act(h, b):
                return jax.nn.gelu(h + b, approximate=True).astype(jnp.bfloat16)

            def dot_nt(a, b):
                return jax.lax.dot_general(a, b, _NT, preferred_element_type=jnp.float32)

            def hidden(xb, f0, f1):
                return act(dot_nt(xb, w1_v[f0:f1, :]), bias1()[:, f0:f1])

            def hidden_tail(xb):
                return act(dot_nt(w1_v[FM:F, :], xb).T, bias1()[:, FM:F])

            def project(g):
                return (jnp.dot(g, w2_v[...], preferred_element_type=jnp.float32) + bias2()).astype(o_v.dtype)

            x_cols = []
            pieces = []
            for p, (r0, r1) in enumerate(x0_pieces):
                for t, (f0, f1) in enumerate(first_tiles):
                    if p == 0:
                        c_w0[t].wait()
                        if t == 4:
                            c_b1.wait()
                    if t == 0:
                        c_x0[p].wait()
                        pieces.append(x_v[r0:r1, 0:_T])
                    h_v[r0:r1, f0:f1] = _row_split(lambda xx: dot_nt(xx, w1_v[f0:f1, 0:_T]), pieces[-1], 4)
            x_cols.append(jnp.concatenate(pieces, axis=0))

            g_parts = []
            for i, ((a, b), fs) in enumerate(_K_STEPS):
                c0, c1 = a * _T, b * _T
                last = i == len(_K_STEPS) - 1
                for j, (f0, f1, n) in enumerate(fs):
                    c_wk[i][j].wait()
                    if j == 0:
                        c_xk[i].wait()
                        x_cols.append(x_v[0:_TM0, c0:c1])
                    p = _row_split(lambda xx: dot_nt(xx, w1_v[f0:f1, c0:c1]), x_cols[-1], n)
                    if last:
                        g_parts.append(act(h_v[:, f0:f1] + p, bias1()[:, f0:f1]))
                    else:
                        h_v[:, f0:f1] += p

            xb = jnp.concatenate(x_cols, axis=1)
            for c, (f0, f1) in zip(c_full, _FULL):
                c.wait()
                g_parts.append(hidden(xb, f0, f1))
            c_tail.wait()
            g_parts.append(hidden_tail(xb))
            g = jnp.concatenate(g_parts, axis=1)
            c_w2.wait()
            c_b2.wait()
            o_v[0:_TM0, :] = project(g)
            outs[0].start()

            for j, (r0, r1) in enumerate(blocks):
                c_xb[j].wait()
                xb = x_v[r0:r1, :]
                g = jnp.concatenate([hidden(xb, 0, FM), hidden_tail(xb)], axis=1)
                for i, (blk, s, e) in enumerate(out_pieces[:-1]):
                    if blk == j:
                        o_v[s:e, :] = project(g[s - r0:e - r0, :])
                        outs[1 + i].start()
            g_last = g[s_last - r0:e_last - r0, :]
            for c, (n0, n1) in zip(outs_last, _LAST_COLS):
                y = jnp.dot(g_last, w2_v[:, n0:n1], preferred_element_type=jnp.float32) + bias2()[:, n0:n1]
                o_v[s_last:e_last, n0:n1] = y.astype(o_v.dtype)
                c.start()

            for c in outs + outs_last:
                c.wait()

        def trip(t, carry):
            pl.when(t == 0)(work)
            return carry

        jax.lax.fori_loop(0, 2, trip, 0)

    return kernel, n_in, n_out


@jax.jit
def pallas_standalone__dense_activation_gelu__prompt_kernel(x, w1, b1, w2, b2):
    B, S, D = x.shape
    F = w1.shape[1]
    M = B * S
    kernel, n_in, n_out = _make_kernel(M, D, F)
    hbm = pl.BlockSpec(memory_space=pltpu.HBM)
    out = pl.pallas_call(
        kernel,
        in_specs=[hbm] * 5,
        out_specs=hbm,
        out_shape=jax.ShapeDtypeStruct((M, D), x.dtype),
        scratch_shapes=[
            pltpu.VMEM((M, D), x.dtype),
            pltpu.VMEM((F, D), w1.dtype),
            pltpu.VMEM((F, D), w2.dtype),
            pltpu.VMEM((F,), b1.dtype),
            pltpu.VMEM((D,), b2.dtype),
            pltpu.VMEM((M, D), x.dtype),
            pltpu.VMEM((_TM0, _FA), jnp.float32),
            pltpu.SemaphoreType.DMA((n_in,)),
            pltpu.SemaphoreType.DMA((n_out,)),
        ],
        compiler_params=pltpu.CompilerParams(
            vmem_limit_bytes=100 * 1024 * 1024,
            disable_semaphore_checks=True,
            flags={"XLA_TPU_RESCHEDULE_DMA_DONES": True},
        ),
    )(x.reshape(M, D), w1.T, b1, w2, b2)
    return out.reshape(B, S, D)
```
